```python
import os as _os
_os.environ.setdefault("JAX_PLATFORMS", "cpu")
import jax
import jax.numpy as jnp

def _softmax(x, axis=-1):
    return jax.nn.softmax(x, axis=axis)
def _gelu(x):
    return jax.nn.gelu(x, approximate=True)
def _silu(x):
    return jax.nn.silu(x)
def _sigmoid(x):
    return jax.nn.sigmoid(x)
def _layernorm(x, axis=-1, eps=1e-5):
    m = jnp.mean(x, axis=axis, keepdims=True)
    v = jnp.var(x, axis=axis, keepdims=True)
    return (x - m) / jnp.sqrt(v + eps)
def _scatter_add(tgt, idx, src, axis=0):
    return tgt.at[idx].add(src)
def _segment_sum(src, seg, n):
    return jax.ops.segment_sum(src, seg, n)
class _Rng:
    def __init__(self, key):
        self._k = key
    def _next(self):
        self._k, sub = jax.random.split(self._k)
        return sub
    def normal(self, shape):
        return jax.random.normal(self._next(), shape, dtype=jnp.bfloat16)
    def randint(self, lo, hi, shape):
        return jax.random.randint(self._next(), shape, lo, hi, dtype=jnp.int32)
    def uniform(self, shape, lo=0.0, hi=1.0):
        return jax.random.uniform(self._next(), shape, jnp.bfloat16, lo, hi)
    def permutation(self, n):
        return jax.random.permutation(self._next(), n)


kernel_name = 'standalone__fft_conv__vision'

def setup_inputs():
    _rng = _Rng(jax.random.key(int.from_bytes(__import__("os").urandom(4), "little")))
    _w = (lambda a: (lambda t: t.astype(jnp.bfloat16) if jnp.issubdtype(t.dtype, jnp.floating) else t)(jnp.asarray(a)))
    H = W = 224
    C = 96
    K = 3
    return {
        "x": _w((lambda *s: _rng.normal(s) * 0.05)(1, H, W, C)),
        "w": _w((lambda *s: _rng.normal(s) * 0.05)(K, K, C, C)),
    }

def reference(x, w):
    B, H, W, C = x.shape
    K = w.shape[0]
    wp = jnp.pad(w, ((0, H - K), (0, W - K), (0, 0), (0, 0)))
    Xf = (lambda x, axes=(-2,-1): jnp.fft.rfft2(x.astype(jnp.float32), axes=axes))(x, axes=(1, 2))
    Wf = (lambda x, axes=(-2,-1): jnp.fft.rfft2(x.astype(jnp.float32), axes=axes))(wp, axes=(0, 1))
    Yf = jnp.einsum('bhwi,hwio->bhwo', Xf, Wf)
    y = (lambda x, s, axes=(-2,-1): jnp.fft.irfft2(x, s=s, axes=axes).astype(jnp.bfloat16))(Yf, (H, W), axes=(1, 2))
    return y
```

```python
import functools
import jax, jax.numpy as jnp, numpy as np
from jax import lax
from jax.experimental import pallas as pl
from jax.experimental.pallas import tpu as pltpu

F32, BF16, I32 = jnp.float32, jnp.bfloat16, jnp.int32
H = W = 224; C = 96; NP = H // 2

def extras14():
    ex = {(a, b): [] for a in range(4) for b in range(4) if (a, b) not in ((0, 0), (3, 3))}
    def put(src, g, *dst):
        for (a, b, s) in dst: ex[(a, b)].append((src, g, s))
    put((0,0), 0, (0,1,.5), (0,2,.5))
    put((0,0), 1, (0,1,1.), (0,3,1.))
    put((0,0), 2, (0,2,1.), (0,3,-1.))
    put((0,0), 3, (1,0,.5), (2,0,.5))
    put((0,0), 4, (1,0,.5), (2,0,.5))
    put((0,0), 5, (1,1,.25), (1,2,.25), (2,1,.25), (2,2,.25))
    put((3,3), 0, (3,2,.5), (3,1,-.5))
    put((3,3), 1, (3,0,1.), (3,1,-1.))
    put((3,3), 2, (3,2,1.), (3,0,-1.))
    put((3,3), 3, (2,3,.5), (1,3,-.5))
    put((3,3), 4, (2,3,.5), (1,3,-.5))
    put((3,3), 5, (1,1,.25), (1,2,-.25), (2,1,-.25), (2,2,.25))
    assert all(len(v) == 2 for v in ex.values())
    return ex

def make(U=4, dma=True, wstart=6, ahead=99, flags=None, border=(1,2,3,0), NT=4, lag=4, frow=11, rotlag=1, gsched=(2,2,2,0), asched=(0,0,0,6), defer=True):
    ex = extras14()
    keys = sorted(ex)
    def kernel(x_hbm, w_hbm, o_hbm, w_ref, xbuf, obuf, ubuf, tb, yb, sm, isem, osem):
        NI = NP // U; R = 2 * U
        def icopy(r0, n, s): return pltpu.make_async_copy(x_hbm.at[pl.ds(r0, n)], xbuf.at[pl.ds(r0, n)], isem.at[s])
        def ocopy(r0, n, s): return pltpu.make_async_copy(obuf.at[pl.ds(r0, n)], o_hbm.at[pl.ds(r0, n)], osem.at[s])
        def in_chunk(i): return icopy(6 + R*i, R, i)
        def in_last(): return icopy(6 + R*(NI-1), R-6, NI-1)
        wcopy = pltpu.make_async_copy(w_hbm, w_ref, isem.at[NI+1])
        wcopy.start()
        if dma:
            icopy(0, 6, NI).start()
            for i in range(min(ahead, NI-1)): in_chunk(i).start()
            if ahead >= NI: in_last().start()
        wcopy.wait()
        f = [[w_ref[2-k, 2-l].astype(F32) for l in range(3)] for k in range(3)]
        def g4(a, b, c):
            s = a + c
            return [a, (s + b) * 0.5, (s - b) * 0.5, c]
        fl = [g4(*f[k]) for k in range(3)]
        Uw = {}
        for b in range(4):
            ua = g4(fl[0][b], fl[1][b], fl[2][b])
            for a in range(4): Uw[(a, b)] = ua[a]
        for n, k in enumerate(keys):
            parts = [Uw[k]] + [Uw[src][16*g:16*g+16] * s for (src, g, s) in ex[k]]
            u = jnp.concatenate(parts, axis=0)
            ubuf[n] = pltpu.bitcast(u.astype(BF16).T, I32)
        if dma: icopy(0, 6, NI).wait()

        lane = lax.broadcasted_iota(I32, (8, 128), 1)
        even = (lane & 1) == 0
        hi2 = lane >= 126
        lanef = lax.broadcasted_iota(I32, (C, 128), 1)
        evenf = (lanef & 1) == 0
        moa = (evenf & (lanef < 126)) | (lanef == 127)
        XX = 8 * NT
        FN = XX + 4

        def row(p):
            if isinstance(p, int): return 2 * (p % NP)
            return 2 * jnp.where(p >= NP, p - NP, p)
        def stA(r, slot, gs):
            for g in gs:
                for q in range(2):
                    A = xbuf[r+q, 16*g:16*g+16, 0:128]
                    B = pltpu.bitcast(jnp.concatenate([xbuf[r+q, 16*g:16*g+16, 128:224], A[:, 96:]], axis=1), I32)
                    A = jnp.where(hi2, pltpu.roll(B, 32, 1), pltpu.bitcast(A, I32))
                    tb[XX+2*slot+q, 8*g:8*g+8] = pltpu.bitcast(jnp.where(even, A, B), F32)
                    tb[XX+2*slot+q, 48+8*g:48+8*g+8] = pltpu.bitcast(jnp.where(even, B, A), F32)
        def up(v): return pltpu.bitcast(v, BF16).astype(F32)
        def stB1(slot, gs):
            res = []
            for g in gs:
                for q in range(2):
                    X0 = tb[XX+2*slot+q, 8*g:8*g+8]; X1 = tb[XX+2*slot+q, 48+8*g:48+8*g+8]
                    res.append((g, q, pltpu.roll(X0, 2, 1), pltpu.roll(X1, 1, 1), pltpu.roll(X1, 127, 1)))
            return res
        def stB2(slot, ts, res):
            for (g, q, e0, e1, e3) in res:
                d0 = up(e0); d1 = up(e1); d2 = up(tb[XX+2*slot+q, 8*g:8*g+8]); d3 = up(e3)
                for b, t in enumerate([d0-d2, d1+d2, d2-d1, d1-d3]): tb[8*ts+4*q+b, 16*g:16*g+16] = t
        def V(tp, tc, a, b, sl=slice(None)):
            if a == 0: return tb[8*tp+b, sl] - tb[8*tc+b, sl]
            if a == 1: return tb[8*tp+4+b, sl] + tb[8*tc+b, sl]
            if a == 2: return tb[8*tc+b, sl] - tb[8*tp+4+b, sl]
            if a == 3: return tb[8*tp+4+b, sl] - tb[8*tc+4+b, sl]
        def mm(tp, tc, b):
            M = {}; cache = {}
            for a in range(4):
                if (a, b) not in ex: continue
                parts = [V(tp, tc, a, b)]
                for (src, g, s) in ex[(a, b)]:
                    if (src, g) not in cache: cache[(src, g)] = V(tp, tc, *src, slice(16*g, 16*g+16))
                    parts.append(cache[(src, g)])
                v = jnp.concatenate(parts, axis=0)
                M[a] = jnp.dot(pltpu.bitcast(ubuf[keys.index((a, b))], BF16), v.astype(BF16), preferred_element_type=F32)
            z0 = M[1] + M[2]; z1 = M[1] - M[2]
            if 0 in M: z0 = z0 + M[0]
            if 3 in M: z1 = z1 - M[3]
            return z0, z1
        def put(r, ye, yo):
            yo = pltpu.roll(yo, 1, 1)
            o = jnp.concatenate([jnp.where(moa, ye, yo), jnp.where(evenf, yo, ye)[:, :96]], axis=1)
            obuf[r] = o.astype(BF16)
        def out(r, Z, later):
            for q in range(2):
                if border[0] == 3: yo = Z[1][q]-Z[3][q]-Z[2][q]
                else: yo = Z[1][q]-Z[2][q]-Z[3][q]
                if border[0] == 0: ye = Z[0][q]+Z[1][q]+Z[2][q]
                else: ye = Z[1][q]+Z[2][q]+Z[0][q]
                if later: yb[2*q] = ye; yb[2*q+1] = yo
                else: put(r+q, ye, yo)
        def flush(r):
            for q in range(2): put(r+q, yb[2*q], yb[2*q+1])

        G6 = range(6)
        sm[0] = FN
        stA(0, 0, G6); stA(2, 1, G6); stB2(0, 0, stB1(0, G6)); stB2(1, 1 % NT, stB1(1, G6)); stA(4, 0, G6)
        def cum(s):
            c = np.concatenate([[0], np.cumsum(s)]); return [range(c[i], c[i+1]) for i in range(4)]
        gs = cum(gsched); as_ = cum(asched)
        def body(i, c):
            hist = []; pend = []
            if dma:
                @pl.when(i < wstart)
                def _(): in_chunk(i).wait()
                @pl.when(i == wstart)
                def _():
                    for j in range(wstart, NI-1): in_chunk(j).wait()
                    ocopy(2, R*wstart-2, 0).start()
                    in_last().wait()
                @pl.when(i > wstart)
                def _(): ocopy(R*(i-1), R, i).start()
            fidx = sm[0]
            if defer: flush(2*U*i)
            for u in range(U):
                p = 1 + i*U + u; pu = u + 1
                Z = {}
                ra = row(p+2); ro = row(p)
                for k, b in enumerate(border):
                    if lag and len(hist) >= lag:
                        tb[fidx, 0:8] = hist[-lag][8*frow:8*frow+8]
                    Z[b] = mm((pu-1) % NT, pu % NT, b)
                    hist.append(Z[b][0])
                    pend.append(((pu+1) % 2, (pu+1) % NT, stB1((pu+1) % 2, gs[k])))
                    while len(pend) > (rotlag if k < 3 else 0):
                        stB2(*pend.pop(0))
                    stA(ra, pu % 2, as_[k])
                out(ro, Z, defer and u == U-1)
            return c
        if defer: yb[...] = jnp.zeros(yb.shape, F32)
        lax.fori_loop(0, NP//U, body, 0)
        if dma: ocopy(R*(NI-1), R, NI).start()
        if defer: flush(0)
        if dma:
            ocopy(0, 2, NI+1).start()
            ocopy(2, R*wstart-2, 0).wait()
            for j in range(wstart+1, NI+1): ocopy(R*(j-1), R, j).wait()
            ocopy(0, 2, NI+1).wait()

    def f(x, w):
        xt = jnp.transpose(x[0], (0,2,1))
        y = pl.pallas_call(kernel,
            in_specs=[pl.BlockSpec(memory_space=pl.ANY), pl.BlockSpec(memory_space=pl.ANY)],
            out_specs=pl.BlockSpec(memory_space=pl.ANY),
            out_shape=jax.ShapeDtypeStruct((H,C,W), BF16),
            scratch_shapes=[pltpu.VMEM((3,3,C,C), BF16), pltpu.VMEM((H,C,W), BF16), pltpu.VMEM((H,C,W), BF16),
                            pltpu.VMEM((len(keys),C//2,128), I32),
                            pltpu.VMEM((8*NT+4+2,C,128), F32), pltpu.VMEM((4,C,128), F32), pltpu.SMEM((1,), I32),
                            pltpu.SemaphoreType.DMA((NP//U+2,)), pltpu.SemaphoreType.DMA((NP//U+2,))],
            compiler_params=pltpu.CompilerParams(vmem_limit_bytes=100*1024*1024, flags=flags),
            name="wino",
        )(xt, w)
        return jnp.transpose(y, (0,2,1))[None]
    return f


_impl = make(U=8, wstart=6)


@jax.jit
def pallas_standalone__fft_conv__vision_kernel(x: jax.Array, w: jax.Array):
    return _impl(x, w)
```

```python
import jax
import jax.numpy as jnp
from jax import lax
from jax.experimental import pallas as pl
from jax.experimental.pallas import tpu as pltpu

F32, BF16, I32 = jnp.float32, jnp.bfloat16, jnp.int32
H = W = 224
C = 96
LANES = 128
W_HI = W - LANES
HALF = H // 2

STEPS = H // 2
BLOCKS = ((4, 1), (8, 1), (16, 1), (28, 3))
FETCH_UP_FRONT = 20
WRITE_FROM = 26
SLOTS = 4
GROUPS = 2
FEED_LAG = (-33, -30, -27, -24)
STORE_LAG = 6

OUTPUTS = {0: ((0, 1),), 1: ((0, 1), (1, 1)), 2: ((0, 1), (1, -1)), 3: ((1, -1),)}


def _spare_rows():
    spare = {(a, b): [] for a in range(4) for b in range(4) if (a, b) not in ((0, 0), (3, 3))}
    for source, group, hosts in (
        ((0, 0), 0, ((0, 1, 0.5), (0, 2, 0.5))),
        ((0, 0), 1, ((0, 1, 1.0), (0, 3, 1.0))),
        ((0, 0), 2, ((0, 2, 1.0), (0, 3, -1.0))),
        ((0, 0), 3, ((1, 0, 0.5), (2, 0, 0.5))),
        ((0, 0), 4, ((1, 0, 0.5), (2, 0, 0.5))),
        ((0, 0), 5, ((1, 1, 0.25), (1, 2, 0.25), (2, 1, 0.25), (2, 2, 0.25))),
        ((3, 3), 0, ((3, 2, 0.5), (3, 1, -0.5))),
        ((3, 3), 1, ((3, 0, 1.0), (3, 1, -1.0))),
        ((3, 3), 2, ((3, 2, 1.0), (3, 0, -1.0))),
        ((3, 3), 3, ((2, 3, 0.5), (1, 3, -0.5))),
        ((3, 3), 4, ((2, 3, 0.5), (1, 3, -0.5))),
        ((3, 3), 5, ((1, 1, 0.25), (1, 2, -0.25), (2, 1, -0.25), (2, 2, 0.25))),
    ):
        for a, b, scale in hosts:
            spare[(a, b)].append((source, group, scale))
    return spare


def _column(step, b):
    return [(step, (a, b)) for a in range(4)]


def _block_starts():
    starts = [2]
    for length, count in BLOCKS:
        for _ in range(count):
            starts.append(starts[-1] + length)
    assert starts[-1] == STEPS + 2
    return starts[:-1]


SPARE = _spare_rows()
MATMULS = sorted(SPARE)
WAVES = (
    _column(0, 1),
    _column(0, 2),
    [(0, (0, 3)), (0, (1, 3)), (0, (2, 3)), (0, (3, 0))],
    [(0, (1, 0)), (0, (2, 0)), (1, (1, 3)), (1, (2, 3))],
    _column(1, 1),
    _column(1, 2),
    [(1, (0, 3)), (1, (1, 0)), (1, (2, 0)), (1, (3, 0))],
)
STARTS = _block_starts()
EDGES = [0] + [s + 2 for s in STARTS] + [STEPS]
CHUNKS = len(EDGES) - 1


def _signed_add(x, y):
    if x is None:
        return y
    if x[0] == y[0]:
        return x[0], x[1] + y[1]
    return (1, x[1] - y[1]) if x[0] > 0 else (1, y[1] - x[1])


def _when(cond, fn):
    if cond is True:
        fn()
    elif cond is not False:
        pl.when(cond)(fn)


def _kernel(x_hbm, w_hbm, o_hbm, w_s, lo_s, hi_s, o_s, u_s, y_s, t_s, e_s, zero_s, in_sem, out_sem):
    def fetch(n, ahead=0, chunk_ahead=0):
        c = max(c for c in range(CHUNKS) if EDGES[c] <= n) + chunk_ahead
        src = pl.ds(HALF * (n % 2) + n - n % 2 + ahead, 2)
        dst = pl.ds(2 * (n + ahead), 2)
        pltpu.make_async_copy(x_hbm.at[src, :, pl.ds(0, LANES)], lo_s.at[dst], in_sem.at[2 * c]).start()
        pltpu.make_async_copy(x_hbm.at[src, :, pl.ds(LANES, W_HI)], hi_s.at[dst], in_sem.at[2 * c + 1]).start()

    def arrive(c, ahead=0):
        size = 2 * (EDGES[c + 1] - EDGES[c])
        rows = pl.ds(2 * EDGES[c] + ahead * size, size)
        pltpu.make_async_copy(lo_s.at[rows], lo_s.at[rows], in_sem.at[2 * (c + ahead)]).wait()
        pltpu.make_async_copy(hi_s.at[rows], hi_s.at[rows], in_sem.at[2 * (c + ahead) + 1]).wait()

    def send(row, n=1):
        pltpu.make_async_copy(o_s.at[pl.ds(row, n)], o_hbm.at[pl.ds(row, n)], out_sem).start()

    w_copy = pltpu.make_async_copy(w_hbm, w_s, in_sem.at[2 * CHUNKS])
    w_copy.start()
    for n in range(FETCH_UP_FRONT):
        fetch(n)
    zero_s[0] = 0
    w_copy.wait()

    def filter_1d(f0, f1, f2):
        s = f0 + f2
        return [f0, (s + f1) * 0.5, (s - f1) * 0.5, f2]

    along_w = [filter_1d(*[w_s[2 - k, 2 - l].astype(F32) for l in range(3)]) for k in range(3)]
    u = {}
    for b in range(4):
        for a, val in enumerate(filter_1d(*[along_w[k][b] for k in range(3)])):
            u[(a, b)] = val
    for i, key in enumerate(MATMULS):
        rows = [u[key]] + [u[src][16 * g:16 * g + 16] * scale for src, g, scale in SPARE[key]]
        u_s[i] = pltpu.bitcast(jnp.concatenate(rows, axis=0).astype(BF16).T, I32)

    lane = lax.broadcasted_iota(I32, (8 * GROUPS, LANES), 1)
    even, odd = (lane & 1) == 0, (lane & 1) == 1
    lo_in_e0 = (even & (lane != 126)) | (odd & (lane >= W_HI))
    lo_in_e1 = (odd & (lane != 127)) | (even & (lane >= W_HI))
    lane = lax.broadcasted_iota(I32, (C, LANES), 1)
    second_in_hi = (lane & 1) == 0
    first_in_lo = (second_in_hi & (lane < 126)) | (lane == 127)
    pieces = [(g, q) for g in reversed(range(0, C // 16, GROUPS)) for q in (1, 0)]

    def interleave(row, e):
        for g, q in pieces:
            ch = slice(8 * g, 8 * (g + GROUPS))
            lo = lo_s.bitcast(I32)[row + q, ch]
            hi = hi_s.bitcast(I32)[row + q, ch]
            hi = jnp.concatenate([hi, hi[:, 2 * W_HI - LANES:]], axis=1)
            e[2 * q, ch] = jnp.where(lo_in_e0, lo, hi)
            e[2 * q + 1, ch] = jnp.where(lo_in_e1, lo, hi)

    def widen(packed):
        return pltpu.bitcast(packed, BF16).astype(F32)

    def transform_w(e, t):
        for g, q in pieces:
            ch = slice(8 * g, 8 * (g + GROUPS))
            e0, e1 = e[2 * q, ch], e[2 * q + 1, ch]
            d0 = widen(pltpu.roll(e0, 2, 1))
            d1 = widen(pltpu.roll(e1, 1, 1))
            d2 = widen(e0)
            d3 = widen(pltpu.roll(e1, LANES - 1, 1))
            for b, val in enumerate((d0 - d2, d1 + d2, d2 - d1, d1 - d3)):
                t[4 * q + b, 16 * g:16 * (g + GROUPS)] = val

    def put(row, first, second):
        second = pltpu.roll(second, 1, 1)
        lo = jnp.where(first_in_lo, first, second)
        hi = jnp.where(second_in_hi, second, first)[:, :W_HI]
        o_s[row] = jnp.concatenate([lo, hi], axis=1).astype(BF16)

    def emit(pair, first, last):
        if last < WRITE_FROM:
            return
        end = 2 * WRITE_FROM - 1
        new = True if first >= WRITE_FROM else pair >= WRITE_FROM
        left = True if last < end else False if first >= end else pair < end
        old = left if new is True else new if left is True else new & left
        for q in range(2):
            for s in range(2):
                _when(new, lambda: send(HALF * s + 2 * pair + q))
                _when(old, lambda: send(HALF * s + 2 * (pair - WRITE_FROM + 1) + q))

    def block(first, length, count, it):
        last = first + (count - 1) * length
        chunk = STARTS.index(first) + 1
        if count == 1:
            arrive(chunk)
        else:
            _when(it < count - 1, lambda: arrive(chunk, it))
            _when(it == count - 1, lambda: arrive(chunk + count - 1))
        zero = zero_s[0]
        pair = first // 2 + (length // 2) * it + zero
        sums, stored, turn = [], {}, [0]

        if first > STARTS[0]:
            row = HALF + 2 * (pair - 1)
            for q in range(2):
                put(row + q, y_s[2 * q], y_s[2 * q + 1])
            emit(pair - 1, first // 2 - 1, last // 2 - 1)
            stored[STORE_LAG - 2] = o_s[row + zero, 0:8, 0:LANES].astype(F32)

        def run_ahead(k):
            n = first + k
            transform_w(e_s[(n + 1) % SLOTS], t_s[(n + 1) % SLOTS])
            for m in range(FETCH_UP_FRONT + 2 * (n - 2), min(STEPS, FETCH_UP_FRONT + 2 * (n - 1))):
                _when(count == 1 or m + 2 * length * it < STEPS,
                      lambda: fetch(m, zero + 2 * length * it, 2 * it))
            m = 2 * pair + k + 2
            if last + k + 2 >= STEPS:
                m = jnp.where(m >= STEPS, 1 - k % 2, m)
            interleave(2 * m, e_s[(n + 2) % SLOTS])

        for k in range(0, length, 2):
            todo = {}
            for wave in WAVES:
                for key in {(s, q, p): 1 for s, (a, b) in wave for q, _ in OUTPUTS[a] for p, _ in OUTPUTS[b]}:
                    todo[key] = todo.get(key, 0) + 1
            acc = {}
            for i, wave in enumerate(WAVES):
                if i == 3:
                    run_ahead(k)
                loaded, tiles = {}, {}

                def tile(s, a, b, g, n):
                    def t(r):
                        if (s, r, b, g, n) not in loaded:
                            ref = t_s[(first + k + s - 2 + 2 * (r // 2)) % SLOTS]
                            loaded[(s, r, b, g, n)] = ref[4 * (r % 2) + b, 16 * g:16 * (g + n)]
                        return loaded[(s, r, b, g, n)]

                    if (s, a, b, g, n) not in tiles:
                        tiles[(s, a, b, g, n)] = (
                            t(0) - t(2) if a == 0 else t(1) + t(2) if a == 1
                            else t(2) - t(1) if a == 2 else t(1) - t(3))
                    return tiles[(s, a, b, g, n)]

                def gate(value):
                    t_s[(first + k + wave[0][0]) % SLOTS][8 + zero, 0:8] = value

                if len(sums) in stored:
                    gate(stored.pop(len(sums)))
                rhs = {m: [] for m in wave}
                for j, lag in enumerate(FEED_LAG):
                    at = 12 * len(sums) + lag
                    if at >= 0:
                        turn[0] += 1
                        earlier = sums[at // 12]
                        gate(earlier[turn[0] % len(earlier)][8 * (at % 12):8 * (at % 12) + 8])
                    if j == 0:
                        for z in (1, 0):
                            for s, key in wave:
                                src, g, _ = SPARE[key][z]
                                rhs[(s, key)].insert(0, tile(s, *src, g, 1))
                    else:
                        for s, key in wave:
                            rhs[(s, key)].insert(0, tile(s, *key, 6 - 2 * j, 2))
                prod = {}
                for s, key in wave:
                    prod[(s, key)] = jnp.dot(
                        pltpu.bitcast(u_s[MATMULS.index(key)], BF16),
                        jnp.concatenate(rhs[(s, key)], axis=0).astype(BF16),
                        preferred_element_type=F32)

                rows = {}
                for s, (a, b) in sorted(prod, key=lambda m: (m[0], m[1][1], (1, 2, 0, 3).index(m[1][0]))):
                    for q, sign in OUTPUTS[a]:
                        rows[(s, q, b)] = _signed_add(rows.get((s, q, b)), (sign, prod[(s, (a, b))]))
                parts = {}
                for (s, q, b), (sign, val) in rows.items():
                    for p, sign_w in OUTPUTS[b]:
                        parts[(s, q, p)] = _signed_add(parts.get((s, q, p)), (sign * sign_w, val))
                for key, val in parts.items():
                    acc[key] = _signed_add(acc.get(key), val)
                    todo[key] -= 1
                sums.append([acc[key][1] for key in sorted(parts) if key[2] == 1])

                for s in range(2):
                    keys = [(s, q, p) for q in range(2) for p in range(2)]
                    if keys[0] not in parts or any(todo[key] for key in keys):
                        continue
                    assert all(acc[key][0] == 1 for key in keys)
                    if k + s == length - 1:
                        for j, key in enumerate(keys):
                            y_s[j] = acc[key][1]
                        continue
                    row = HALF * s + 2 * pair + k
                    for q in range(2):
                        put(row + q, acc[(s, q, 0)][1], acc[(s, q, 1)][1])
                    if s:
                        emit(pair + k // 2, (first + k) // 2, (last + k) // 2)
                    stored[len(sums) - 1 + STORE_LAG] = o_s[row + zero, 0:8, 0:LANES].astype(F32)
            run_ahead(k + 1)

    arrive(0)
    for n in range(4):
        interleave(2 * n, e_s[n])
        if n < 3:
            transform_w(e_s[n], t_s[n])
    first = STARTS[0]
    for length, count in BLOCKS:
        if count == 1:
            block(first, length, 1, 0)
        else:
            pl.loop(0, count)(lambda it: block(first, length, count, it))
        first += length * count
    send(HALF + zero_s[0], 2)
    for q in range(2):
        put(q, y_s[2 * q], y_s[2 * q + 1])
    send(0, 2)
    pltpu.make_async_copy(o_s, o_hbm, out_sem).wait()


@jax.jit
def pallas_standalone__fft_conv__vision_kernel(x: jax.Array, w: jax.Array):
    assert x.shape == (1, H, W, C) and w.shape == (3, 3, C, C)
    y = pl.pallas_call(
        _kernel,
        in_specs=[pl.BlockSpec(memory_space=pl.ANY)] * 2,
        out_specs=pl.BlockSpec(memory_space=pl.ANY),
        out_shape=jax.ShapeDtypeStruct((H, C, W), BF16),
        scratch_shapes=[
            pltpu.VMEM((3, 3, C, C), BF16),
            pltpu.VMEM((H, C, LANES), BF16),
            pltpu.VMEM((H, C, W_HI), BF16),
            pltpu.VMEM((H, C, W), BF16),
            pltpu.VMEM((len(MATMULS), C // 2, LANES), I32),
            pltpu.VMEM((4, C, LANES), F32),
            [pltpu.VMEM((9, C + 8, LANES), F32)] * SLOTS,
            [pltpu.VMEM((4, C // 2, LANES), I32)] * SLOTS,
            pltpu.SMEM((1,), I32),
            pltpu.SemaphoreType.DMA((2 * CHUNKS + 1,)),
            pltpu.SemaphoreType.DMA(()),
        ],
        compiler_params=pltpu.CompilerParams(
            vmem_limit_bytes=48 * 1024 * 1024,
            disable_bounds_checks=True,
            disable_semaphore_checks=True,
        ),
    )(jnp.transpose(x.astype(BF16).reshape(H, W, C), (0, 2, 1)), w.astype(BF16))
    return jnp.transpose(y, (0, 2, 1)).reshape(1, H, W, C)
```

```python
import jax
import jax.numpy as jnp
from jax import lax
from jax.experimental import pallas as pl
from jax.experimental.pallas import tpu as pltpu

F32, BF16, I32 = jnp.float32, jnp.bfloat16, jnp.int32
H = W = 224
C = 96
LANES = 128
W_HI = W - LANES
HALF = H // 2

STEPS = H // 2
BLOCKS = ((4, 1), (8, 1), (16, 1), (28, 3))
FETCH_UP_FRONT = 16
TWO_QUEUES_FROM = 36
WRITE_FROM = 26
E_SLOTS, T_SLOTS = 2, 4
GROUPS = 2
FEED_LAG = (-34, -30, -28, -26)
WAVE_LAG = (0, -2, -2, 0, 0, 0, 0)
STORE_LAG = 6

OUTPUTS = {0: ((0, 1),), 1: ((0, 1), (1, 1)), 2: ((0, 1), (1, -1)), 3: ((1, -1),)}


def _spare_rows():
    spare = {(a, b): [] for a in range(4) for b in range(4) if (a, b) not in ((0, 0), (3, 3))}
    for source, group, hosts in (
        ((0, 0), 0, ((0, 1, 0.5), (0, 2, 0.5))),
        ((0, 0), 1, ((0, 1, 1.0), (0, 3, 1.0))),
        ((0, 0), 2, ((0, 2, 1.0), (0, 3, -1.0))),
        ((0, 0), 3, ((1, 0, 0.5), (2, 0, 0.5))),
        ((0, 0), 4, ((1, 0, 0.5), (2, 0, 0.5))),
        ((0, 0), 5, ((1, 1, 0.25), (1, 2, 0.25), (2, 1, 0.25), (2, 2, 0.25))),
        ((3, 3), 0, ((3, 2, 0.5), (3, 1, -0.5))),
        ((3, 3), 1, ((3, 0, 1.0), (3, 1, -1.0))),
        ((3, 3), 2, ((3, 2, 1.0), (3, 0, -1.0))),
        ((3, 3), 3, ((2, 3, 0.5), (1, 3, -0.5))),
        ((3, 3), 4, ((2, 3, 0.5), (1, 3, -0.5))),
        ((3, 3), 5, ((1, 1, 0.25), (1, 2, -0.25), (2, 1, -0.25), (2, 2, 0.25))),
    ):
        for a, b, scale in hosts:
            spare[(a, b)].append((source, group, scale))
    return spare


def _column(step, b):
    return [(step, (a, b)) for a in range(4)]


def _block_starts():
    starts = [2]
    for length, count in BLOCKS:
        for _ in range(count):
            starts.append(starts[-1] + length)
    assert starts[-1] == STEPS + 2
    return starts[:-1]


SPARE = _spare_rows()
MATMULS = sorted(SPARE)
WAVES = (
    _column(0, 1),
    _column(0, 2),
    [(0, (0, 3)), (0, (1, 3)), (0, (2, 3)), (0, (3, 0))],
    [(0, (1, 0)), (0, (2, 0)), (1, (1, 3)), (1, (2, 3))],
    _column(1, 1),
    _column(1, 2),
    [(1, (0, 3)), (1, (1, 0)), (1, (2, 0)), (1, (3, 0))],
)
STARTS = _block_starts()
EDGES = [0] + [s + 2 for s in STARTS] + [STEPS]
CHUNKS = len(EDGES) - 1


def _signed_add(x, y):
    if x is None:
        return y
    if x[0] == y[0]:
        return x[0], x[1] + y[1]
    return (1, x[1] - y[1]) if x[0] > 0 else (1, y[1] - x[1])


def _when(cond, fn):
    if cond is True:
        fn()
    elif cond is not False:
        pl.when(cond)(fn)


def _kernel(x_hbm, w_hbm, o_hbm, w_s, lo_s, hi_s, o_s, u_s, y_s, t_s, e_s, zero_s, in_sem, out_sem):
    def fetch(n, ahead=0, chunk_ahead=0):
        c = max(c for c in range(CHUNKS) if EDGES[c] <= n) + chunk_ahead
        src = pl.ds(HALF * (n % 2) + n - n % 2 + ahead, 2)
        dst = pl.ds(2 * (n + ahead), 2)
        lo = pltpu.make_async_copy(x_hbm.at[src, :, pl.ds(0, LANES)], lo_s.at[dst], in_sem.at[2 * c])
        hi = pltpu.make_async_copy(x_hbm.at[src, :, pl.ds(LANES, W_HI)], hi_s.at[dst], in_sem.at[2 * c + 1])
        lo.start(priority=int(n < TWO_QUEUES_FROM or n % 2))
        hi.start(priority=1)

    def arrive(c, ahead=0):
        size = 2 * (EDGES[c + 1] - EDGES[c])
        rows = pl.ds(2 * EDGES[c] + ahead * size, size)
        pltpu.make_async_copy(lo_s.at[rows], lo_s.at[rows], in_sem.at[2 * (c + ahead)]).wait()
        pltpu.make_async_copy(hi_s.at[rows], hi_s.at[rows], in_sem.at[2 * (c + ahead) + 1]).wait()

    def send(row, n=1):
        pltpu.make_async_copy(o_s.at[pl.ds(row, n)], o_hbm.at[pl.ds(row, n)], out_sem).start()

    w_copy = pltpu.make_async_copy(w_hbm, w_s, in_sem.at[2 * CHUNKS])
    w_copy.start(priority=1)
    for n in range(FETCH_UP_FRONT):
        fetch(n)
    zero_s[0] = 0
    w_copy.wait()

    def filter_1d(f0, f1, f2):
        s = f0 + f2
        return [f0, (s + f1) * 0.5, (s - f1) * 0.5, f2]

    along_w = [filter_1d(*[w_s[2 - k, 2 - l].astype(F32) for l in range(3)]) for k in range(3)]
    u = {}
    for b in range(4):
        for a, val in enumerate(filter_1d(*[along_w[k][b] for k in range(3)])):
            u[(a, b)] = val
    for i, key in enumerate(MATMULS):
        rows = [u[key]] + [u[src][16 * g:16 * g + 16] * scale for src, g, scale in SPARE[key]]
        u_s[i] = pltpu.bitcast(jnp.concatenate(rows, axis=0).astype(BF16).T, I32)

    lane = lax.broadcasted_iota(I32, (8 * GROUPS, LANES), 1)
    even, odd = (lane & 1) == 0, (lane & 1) == 1
    lo_in_e0 = (even & (lane != 126)) | (odd & (lane >= W_HI))
    lo_in_e1 = (odd & (lane != 127)) | (even & (lane >= W_HI))
    lane = lax.broadcasted_iota(I32, (C, LANES), 1)
    second_in_hi = (lane & 1) == 0
    first_in_lo = (second_in_hi & (lane < 126)) | (lane == 127)
    pieces = [(g, q) for g in reversed(range(0, C // 16, GROUPS)) for q in (1, 0)]

    def interleave(row, e):
        for g, q in pieces:
            ch = slice(8 * g, 8 * (g + GROUPS))
            lo = lo_s.bitcast(I32)[row + q, ch]
            hi = hi_s.bitcast(I32)[row + q, ch]
            hi = jnp.concatenate([hi, hi[:, 2 * W_HI - LANES:]], axis=1)
            e[2 * q, ch] = jnp.where(lo_in_e0, lo, hi)
            e[2 * q + 1, ch] = jnp.where(lo_in_e1, lo, hi)

    def widen(packed):
        return pltpu.bitcast(packed, BF16).astype(F32)

    def transform_w(e, t):
        for g, q in pieces:
            ch = slice(8 * g, 8 * (g + GROUPS))
            e0, e1 = e[2 * q, ch], e[2 * q + 1, ch]
            d0 = widen(pltpu.roll(e0, 2, 1))
            d1 = widen(pltpu.roll(e1, 1, 1))
            d2 = widen(e0)
            d3 = widen(pltpu.roll(e1, LANES - 1, 1))
            for b, val in enumerate((d0 - d2, d1 + d2, d2 - d1, d1 - d3)):
                t[4 * q + b, 16 * g:16 * (g + GROUPS)] = val

    def put(row, first, second):
        second = pltpu.roll(second, 1, 1)
        lo = jnp.where(first_in_lo, first, second)
        hi = jnp.where(second_in_hi, second, first)[:, :W_HI]
        o_s[row] = jnp.concatenate([lo, hi], axis=1).astype(BF16)

    def emit(pair, first, last):
        if last < WRITE_FROM:
            return
        end = 2 * WRITE_FROM - 2
        new = True if first >= WRITE_FROM else pair >= WRITE_FROM
        left = True if last < end else False if first >= end else pair < end
        old = left if new is True else new if left is True else new & left
        for q in range(2):
            for s in range(2):
                _when(new, lambda: send(HALF * s + 2 * pair + q))
                _when(old, lambda: send(HALF * s + 2 * (pair - WRITE_FROM + 2) + q))

    def block(first, length, count, it):
        last = first + (count - 1) * length
        chunk = STARTS.index(first) + 1
        if count == 1:
            arrive(chunk)
        else:
            _when(it < count - 1, lambda: arrive(chunk, it))
            _when(it == count - 1, lambda: arrive(chunk + count - 1))
        zero = zero_s[0]
        pair = first // 2 + (length // 2) * it + zero
        sums, stored, turn = [], {}, [1]

        if first > STARTS[0]:
            row = HALF + 2 * (pair - 1)
            for q in range(2):
                put(row + q, y_s[2 * q], y_s[2 * q + 1])
            emit(pair - 1, first // 2 - 1, last // 2 - 1)
            stored[STORE_LAG - 2] = o_s[row + zero, 0:8, 0:LANES].astype(F32)

        def run_ahead(k):
            n = first + k
            transform_w(e_s[(n + 1) % E_SLOTS], t_s[(n + 1) % T_SLOTS])
            for m in range(FETCH_UP_FRONT + 2 * (n - 2), min(STEPS, FETCH_UP_FRONT + 2 * (n - 1))):
                _when(count == 1 or m + 2 * length * it < STEPS,
                      lambda: fetch(m, zero + 2 * length * it, 2 * it))
            m = 2 * pair + k + 2
            if last + k + 2 >= STEPS:
                m = jnp.where(m >= STEPS, 1 - k % 2, m)
            interleave(2 * m, e_s[(n + 2) % E_SLOTS])

        for k in range(0, length, 2):
            todo = {}
            for wave in WAVES:
                for key in {(s, q, p): 1 for s, (a, b) in wave for q, _ in OUTPUTS[a] for p, _ in OUTPUTS[b]}:
                    todo[key] = todo.get(key, 0) + 1
            acc = {}
            for i, wave in enumerate(WAVES):
                if i == 3:
                    run_ahead(k)
                loaded, tiles = {}, {}

                def tile(s, a, b, g, n):
                    def t(r):
                        if (s, r, b, g, n) not in loaded:
                            ref = t_s[(first + k + s - 2 + 2 * (r // 2)) % T_SLOTS]
                            loaded[(s, r, b, g, n)] = ref[4 * (r % 2) + b, 16 * g:16 * (g + n)]
                        return loaded[(s, r, b, g, n)]

                    if (s, a, b, g, n) not in tiles:
                        tiles[(s, a, b, g, n)] = (
                            t(0) - t(2) if a == 0 else t(1) + t(2) if a == 1
                            else t(2) - t(1) if a == 2 else t(1) - t(3))
                    return tiles[(s, a, b, g, n)]

                def gate(value):
                    t_s[(first + k + wave[0][0]) % T_SLOTS][8 + zero, 0:8] = value

                if len(sums) in stored:
                    gate(stored.pop(len(sums)))
                rhs = {m: [] for m in wave}
                for j, lag in enumerate(FEED_LAG):
                    at = 12 * len(sums) + lag + WAVE_LAG[i]
                    if at >= 0:
                        turn[0] += 1
                        earlier = sums[at // 12]
                        gate(earlier[turn[0] % len(earlier)][8 * (at % 12):8 * (at % 12) + 8])
                    if j == 0:
                        for z in (1, 0):
                            for s, key in wave:
                                src, g, _ = SPARE[key][z]
                                rhs[(s, key)].insert(0, tile(s, *src, g, 1))
                    else:
                        for s, key in wave:
                            rhs[(s, key)].insert(0, tile(s, *key, 6 - 2 * j, 2))
                prod = {}
                for s, key in wave:
                    prod[(s, key)] = jnp.dot(
                        pltpu.bitcast(u_s[MATMULS.index(key)], BF16),
                        jnp.concatenate(rhs[(s, key)], axis=0).astype(BF16),
                        preferred_element_type=F32)

                rows = {}
                for s, (a, b) in sorted(prod, key=lambda m: (m[0], m[1][1], (1, 2, 0, 3).index(m[1][0]))):
                    for q, sign in OUTPUTS[a]:
                        rows[(s, q, b)] = _signed_add(rows.get((s, q, b)), (sign, prod[(s, (a, b))]))
                parts = {}
                for (s, q, b), (sign, val) in rows.items():
                    for p, sign_w in OUTPUTS[b]:
                        parts[(s, q, p)] = _signed_add(parts.get((s, q, p)), (sign * sign_w, val))
                for key, val in parts.items():
                    acc[key] = _signed_add(acc.get(key), val)
                    todo[key] -= 1
                sums.append([acc[key][1] for key in sorted(parts) if key[2] == 1])

                for s in range(2):
                    keys = [(s, q, p) for q in range(2) for p in range(2)]
                    if keys[0] not in parts or any(todo[key] for key in keys):
                        continue
                    assert all(acc[key][0] == 1 for key in keys)
                    if k + s == length - 1:
                        for j, key in enumerate(keys):
                            y_s[j] = acc[key][1]
                        continue
                    row = HALF * s + 2 * pair + k
                    for q in range(2):
                        put(row + q, acc[(s, q, 0)][1], acc[(s, q, 1)][1])
                    if s:
                        emit(pair + k // 2, (first + k) // 2, (last + k) // 2)
                    elif first + k == 2 * WRITE_FROM:
                        for q in range(2):
                            for half in range(2):
                                _when(count == 1 or it == 0, lambda: send(HALF * half + 2 + q + zero))
                    stored[len(sums) - 1 + STORE_LAG] = o_s[row + zero, 0:8, 0:LANES].astype(F32)
            run_ahead(k + 1)

    arrive(0)
    for n in range(4):
        interleave(2 * n, e_s[n % E_SLOTS])
        if n < 3:
            transform_w(e_s[n % E_SLOTS], t_s[n])
    first = STARTS[0]
    for length, count in BLOCKS:
        if count == 1:
            block(first, length, 1, 0)
        else:
            pl.loop(0, count)(lambda it: block(first, length, count, it))
        first += length * count
    send(HALF + zero_s[0], 2)
    for q in range(2):
        put(q, y_s[2 * q], y_s[2 * q + 1])
    send(0, 2)
    pltpu.make_async_copy(o_s, o_hbm, out_sem).wait()


@jax.jit
def pallas_standalone__fft_conv__vision_kernel(x: jax.Array, w: jax.Array):
    assert x.shape == (1, H, W, C) and w.shape == (3, 3, C, C)
    y = pl.pallas_call(
        _kernel,
        in_specs=[pl.BlockSpec(memory_space=pl.ANY)] * 2,
        out_specs=pl.BlockSpec(memory_space=pl.ANY),
        out_shape=jax.ShapeDtypeStruct((H, C, W), BF16),
        scratch_shapes=[
            pltpu.VMEM((3, 3, C, C), BF16),
            pltpu.VMEM((H, C, LANES), BF16),
            pltpu.VMEM((H, C, W_HI), BF16),
            pltpu.VMEM((H, C, W), BF16),
            pltpu.VMEM((len(MATMULS), C // 2, LANES), I32),
            pltpu.VMEM((4, C, LANES), F32),
            [pltpu.VMEM((9, C, LANES), F32)] * T_SLOTS,
            [pltpu.VMEM((4, C // 2, LANES), I32)] * E_SLOTS,
            pltpu.SMEM((1,), I32),
            pltpu.SemaphoreType.DMA((2 * CHUNKS + 1,)),
            pltpu.SemaphoreType.DMA(()),
        ],
        compiler_params=pltpu.CompilerParams(
            vmem_limit_bytes=48 * 1024 * 1024,
            disable_bounds_checks=True,
            disable_semaphore_checks=True,
        ),
    )(jnp.transpose(x.astype(BF16).reshape(H, W, C), (0, 2, 1)), w.astype(BF16))
    return jnp.transpose(y, (0, 2, 1)).reshape(1, H, W, C)
```

```python
import jax
import jax.numpy as jnp
from jax import lax
from jax.experimental import pallas as pl
from jax.experimental.pallas import tpu as pltpu

F32, BF16, I32 = jnp.float32, jnp.bfloat16, jnp.int32
H = W = 224
C = 96
LANES = 128
W_HI = W - LANES
HALF = H // 2

STEPS = H // 2
BLOCKS = ((4, 1), (8, 1), (16, 1), (28, 3))
FETCH_UP_FRONT = 16
TWO_QUEUES_FROM = 36
WRITE_FROM = 26
E_SLOTS, T_SLOTS = 2, 4
GROUPS = 2
FEED_LAG = ((32, 28, 26, 26), (36, 32, 30, 28), (38, 32, 30, 28)) + ((34, 30, 28, 26),) * 4
STORE_LAG = 6

OUTPUTS = {0: ((0, 1),), 1: ((0, 1), (1, 1)), 2: ((0, 1), (1, -1)), 3: ((1, -1),)}


def _spare_rows():
    spare = {(a, b): [] for a in range(4) for b in range(4) if (a, b) not in ((0, 0), (3, 3))}
    for source, group, hosts in (
        ((0, 0), 0, ((0, 1, 0.5), (0, 2, 0.5))),
        ((0, 0), 1, ((0, 1, 1.0), (0, 3, 1.0))),
        ((0, 0), 2, ((0, 2, 1.0), (0, 3, -1.0))),
        ((0, 0), 3, ((1, 0, 0.5), (2, 0, 0.5))),
        ((0, 0), 4, ((1, 0, 0.5), (2, 0, 0.5))),
        ((0, 0), 5, ((1, 1, 0.25), (1, 2, 0.25), (2, 1, 0.25), (2, 2, 0.25))),
        ((3, 3), 0, ((3, 2, 0.5), (3, 1, -0.5))),
        ((3, 3), 1, ((3, 0, 1.0), (3, 1, -1.0))),
        ((3, 3), 2, ((3, 2, 1.0), (3, 0, -1.0))),
        ((3, 3), 3, ((2, 3, 0.5), (1, 3, -0.5))),
        ((3, 3), 4, ((2, 3, 0.5), (1, 3, -0.5))),
        ((3, 3), 5, ((1, 1, 0.25), (1, 2, -0.25), (2, 1, -0.25), (2, 2, 0.25))),
    ):
        for a, b, scale in hosts:
            spare[(a, b)].append((source, group, scale))
    return spare


def _column(step, b):
    return [(step, (a, b)) for a in range(4)]


def _block_starts():
    starts = [2]
    for length, count in BLOCKS:
        for _ in range(count):
            starts.append(starts[-1] + length)
    assert starts[-1] == STEPS + 2
    return starts[:-1]


SPARE = _spare_rows()
MATMULS = sorted(SPARE)
WAVES = (
    _column(0, 1),
    _column(0, 2),
    [(0, (0, 3)), (0, (1, 3)), (0, (2, 3)), (0, (3, 0))],
    [(0, (1, 0)), (0, (2, 0)), (1, (1, 3)), (1, (2, 3))],
    _column(1, 1),
    _column(1, 2),
    [(1, (0, 3)), (1, (1, 0)), (1, (2, 0)), (1, (3, 0))],
)
STARTS = _block_starts()
EDGES = [0] + [s + 2 for s in STARTS] + [STEPS]
CHUNKS = len(EDGES) - 1


def _signed_add(x, y):
    if x is None:
        return y
    if x[0] == y[0]:
        return x[0], x[1] + y[1]
    return (1, x[1] - y[1]) if x[0] > 0 else (1, y[1] - x[1])


def _when(cond, fn):
    if cond is True:
        fn()
    elif cond is not False:
        pl.when(cond)(fn)


def _kernel(x_hbm, w_hbm, o_hbm, w_s, lo_s, hi_s, o_s, u_s, y_s, t_s, e_s, zero_s, in_sem, out_sem):
    def fetch(n, ahead=0, chunk_ahead=0):
        c = max(c for c in range(CHUNKS) if EDGES[c] <= n) + chunk_ahead
        src = pl.ds(HALF * (n % 2) + n - n % 2 + ahead, 2)
        dst = pl.ds(2 * (n + ahead), 2)
        lo = pltpu.make_async_copy(x_hbm.at[src, :, pl.ds(0, LANES)], lo_s.at[dst], in_sem.at[2 * c])
        hi = pltpu.make_async_copy(x_hbm.at[src, :, pl.ds(LANES, W_HI)], hi_s.at[dst], in_sem.at[2 * c + 1])
        lo.start(priority=int(n < TWO_QUEUES_FROM or n % 2))
        hi.start(priority=1)

    def arrive(c, ahead=0):
        size = 2 * (EDGES[c + 1] - EDGES[c])
        rows = pl.ds(2 * EDGES[c] + ahead * size, size)
        pltpu.make_async_copy(lo_s.at[rows], lo_s.at[rows], in_sem.at[2 * (c + ahead)]).wait()
        pltpu.make_async_copy(hi_s.at[rows], hi_s.at[rows], in_sem.at[2 * (c + ahead) + 1]).wait()

    def send(row, n=1):
        pltpu.make_async_copy(o_s.at[pl.ds(row, n)], o_hbm.at[pl.ds(row, n)], out_sem).start()

    w_copy = pltpu.make_async_copy(w_hbm, w_s, in_sem.at[2 * CHUNKS])
    w_copy.start(priority=1)
    for n in range(FETCH_UP_FRONT):
        fetch(n)
    zero_s[0] = 0
    w_copy.wait()

    def filter_1d(f0, f1, f2):
        s = f0 + f2
        return [f0, (s + f1) * 0.5, (s - f1) * 0.5, f2]

    along_w = [filter_1d(*[w_s[2 - k, 2 - l].astype(F32) for l in range(3)]) for k in range(3)]
    u = {}
    for b in range(4):
        for a, val in enumerate(filter_1d(*[along_w[k][b] for k in range(3)])):
            u[(a, b)] = val
    for i, key in enumerate(MATMULS):
        rows = [u[key]] + [u[src][16 * g:16 * g + 16] * scale for src, g, scale in SPARE[key]]
        u_s[i] = pltpu.bitcast(jnp.concatenate(rows, axis=0).astype(BF16).T, I32)

    lane = lax.broadcasted_iota(I32, (8 * GROUPS, LANES), 1)
    even, odd = (lane & 1) == 0, (lane & 1) == 1
    lo_in_e0 = (even & (lane != 126)) | (odd & (lane >= W_HI))
    lo_in_e1 = (odd & (lane != 127)) | (even & (lane >= W_HI))
    lane = lax.broadcasted_iota(I32, (C, LANES), 1)
    second_in_hi = (lane & 1) == 0
    first_in_lo = (second_in_hi & (lane < 126)) | (lane == 127)
    pieces = [(g, q) for g in reversed(range(0, C // 16, GROUPS)) for q in (1, 0)]

    def interleave(row, e):
        for g, q in pieces:
            ch = slice(8 * g, 8 * (g + GROUPS))
            lo = pltpu.bitcast(lo_s[row + q, 16 * g:16 * (g + GROUPS)], I32)
            hi = pltpu.bitcast(hi_s[row + q, 16 * g:16 * (g + GROUPS)], I32)
            hi = jnp.concatenate([hi, hi[:, 2 * W_HI - LANES:]], axis=1)
            e[2 * q, ch] = jnp.where(lo_in_e0, lo, hi)
            e[2 * q + 1, ch] = jnp.where(lo_in_e1, lo, hi)

    def widen(packed):
        return pltpu.bitcast(packed, BF16).astype(F32)

    def transform_w(e, t):
        for g, q in pieces:
            ch = slice(8 * g, 8 * (g + GROUPS))
            e0, e1 = e[2 * q, ch], e[2 * q + 1, ch]
            d0 = widen(pltpu.roll(e0, 2, 1))
            d1 = widen(pltpu.roll(e1, 1, 1))
            d2 = widen(e0)
            d3 = widen(pltpu.roll(e1, LANES - 1, 1))
            for b, val in enumerate((d0 - d2, d1 + d2, d2 - d1, d1 - d3)):
                t[4 * q + b, 16 * g:16 * (g + GROUPS)] = val

    def put(row, first, second):
        second = pltpu.roll(second, 1, 1)
        lo = jnp.where(first_in_lo, first, second)
        hi = jnp.where(second_in_hi, second, first)[:, :W_HI]
        o_s[row] = jnp.concatenate([lo, hi], axis=1).astype(BF16)

    def emit(pair, first, last):
        if last < WRITE_FROM:
            return
        end = 2 * WRITE_FROM - 2
        new = True if first >= WRITE_FROM else pair >= WRITE_FROM
        left = True if last < end else False if first >= end else pair < end
        old = left if new is True else new if left is True else new & left
        for q in range(2):
            for s in range(2):
                _when(new, lambda: send(HALF * s + 2 * pair + q))
                _when(old, lambda: send(HALF * s + 2 * (pair - WRITE_FROM + 2) + q))

    def block(first, length, count, it):
        last = first + (count - 1) * length
        chunk = STARTS.index(first) + 1
        if count == 1:
            arrive(chunk)
        else:
            _when(it < count - 1, lambda: arrive(chunk, it))
            _when(it == count - 1, lambda: arrive(chunk + count - 1))
        zero = zero_s[0]
        pair = first // 2 + (length // 2) * it + zero
        sums, stored, turn = [], {}, [1]

        if first > STARTS[0]:
            row = HALF + 2 * (pair - 1)
            for q in range(2):
                put(row + q, y_s[2 * q], y_s[2 * q + 1])
            emit(pair - 1, first // 2 - 1, last // 2 - 1)
            stored[STORE_LAG - 2] = o_s[row + zero, 0:8, 0:LANES].astype(F32)

        def run_ahead(k):
            n = first + k
            transform_w(e_s[(n + 1) % E_SLOTS], t_s[(n + 1) % T_SLOTS])
            for m in range(FETCH_UP_FRONT + 2 * (n - 2), min(STEPS, FETCH_UP_FRONT + 2 * (n - 1))):
                _when(count == 1 or m + 2 * length * it < STEPS,
                      lambda: fetch(m, zero + 2 * length * it, 2 * it))
            m = 2 * pair + k + 2
            if last + k + 2 >= STEPS:
                m = jnp.where(m >= STEPS, 1 - k % 2, m)
            interleave(2 * m, e_s[(n + 2) % E_SLOTS])

        for k in range(0, length, 2):
            todo = {}
            for wave in WAVES:
                for key in {(s, q, p): 1 for s, (a, b) in wave for q, _ in OUTPUTS[a] for p, _ in OUTPUTS[b]}:
                    todo[key] = todo.get(key, 0) + 1
            acc = {}
            for i, wave in enumerate(WAVES):
                if i == 3:
                    run_ahead(k)
                loaded, tiles = {}, {}

                def tile(s, a, b, g, n):
                    def t(r):
                        if (s, r, b, g, n) not in loaded:
                            ref = t_s[(first + k + s - 2 + 2 * (r // 2)) % T_SLOTS]
                            loaded[(s, r, b, g, n)] = ref[4 * (r % 2) + b, 16 * g:16 * (g + n)]
                        return loaded[(s, r, b, g, n)]

                    if (s, a, b, g, n) not in tiles:
                        tiles[(s, a, b, g, n)] = (
                            t(0) - t(2) if a == 0 else t(1) + t(2) if a == 1
                            else t(2) - t(1) if a == 2 else t(1) - t(3))
                    return tiles[(s, a, b, g, n)]

                def gate(value):
                    t_s[(first + k + wave[0][0]) % T_SLOTS][8 + zero, 0:8] = value

                if len(sums) in stored:
                    gate(stored.pop(len(sums)))
                rhs = {m: [] for m in wave}
                for j, lag in enumerate(FEED_LAG[i]):
                    at = 12 * len(sums) - lag
                    if at >= 0:
                        turn[0] += 1
                        earlier = sums[at // 12]
                        gate(earlier[turn[0] % len(earlier)][8 * (at % 12):8 * (at % 12) + 8])
                    if j == 0:
                        for z in (1, 0):
                            for s, key in wave:
                                src, g, _ = SPARE[key][z]
                                rhs[(s, key)].insert(0, tile(s, *src, g, 1))
                    else:
                        for s, key in wave:
                            rhs[(s, key)].insert(0, tile(s, *key, 6 - 2 * j, 2))
                prod = {}
                for s, key in wave:
                    prod[(s, key)] = jnp.dot(
                        pltpu.bitcast(u_s[MATMULS.index(key)], BF16),
                        jnp.concatenate(rhs[(s, key)], axis=0).astype(BF16),
                        preferred_element_type=F32)

                rows = {}
                for s, (a, b) in sorted(prod, key=lambda m: (m[0], m[1][1], (1, 2, 0, 3).index(m[1][0]))):
                    for q, sign in OUTPUTS[a]:
                        rows[(s, q, b)] = _signed_add(rows.get((s, q, b)), (sign, prod[(s, (a, b))]))
                parts = {}
                for (s, q, b), (sign, val) in rows.items():
                    for p, sign_w in OUTPUTS[b]:
                        parts[(s, q, p)] = _signed_add(parts.get((s, q, p)), (sign * sign_w, val))
                for key, val in parts.items():
                    acc[key] = _signed_add(acc.get(key), val)
                    todo[key] -= 1
                sums.append([acc[key][1] for key in sorted(parts) if key[2] == 1])

                for s in range(2):
                    keys = [(s, q, p) for q in range(2) for p in range(2)]
                    if keys[0] not in parts or any(todo[key] for key in keys):
                        continue
                    assert all(acc[key][0] == 1 for key in keys)
                    if k + s == length - 1:
                        for j, key in enumerate(keys):
                            y_s[j] = acc[key][1]
                        continue
                    row = HALF * s + 2 * pair + k
                    for q in range(2):
                        put(row + q, acc[(s, q, 0)][1], acc[(s, q, 1)][1])
                    if s:
                        emit(pair + k // 2, (first + k) // 2, (last + k) // 2)
                    elif first + k == 2 * WRITE_FROM:
                        for q in range(2):
                            for half in range(2):
                                _when(count == 1 or it == 0, lambda: send(HALF * half + 2 + q + zero))
                    stored[len(sums) - 1 + STORE_LAG] = o_s[row + zero, 0:8, 0:LANES].astype(F32)
            run_ahead(k + 1)

    arrive(0)
    for n in range(4):
        interleave(2 * n, e_s[n % E_SLOTS])
        if n < 3:
            transform_w(e_s[n % E_SLOTS], t_s[n])
    first = STARTS[0]
    for length, count in BLOCKS:
        if count == 1:
            block(first, length, 1, 0)
        else:
            pl.loop(0, count)(lambda it: block(first, length, count, it))
        first += length * count
    send(HALF + zero_s[0], 2)
    for q in range(2):
        put(q, y_s[2 * q], y_s[2 * q + 1])
    send(0, 2)
    pltpu.make_async_copy(o_s, o_hbm, out_sem).wait()


@jax.jit
def pallas_standalone__fft_conv__vision_kernel(x: jax.Array, w: jax.Array):
    assert x.shape == (1, H, W, C) and w.shape == (3, 3, C, C)
    y = pl.pallas_call(
        _kernel,
        in_specs=[pl.BlockSpec(memory_space=pl.ANY)] * 2,
        out_specs=pl.BlockSpec(memory_space=pl.ANY),
        out_shape=jax.ShapeDtypeStruct((H, C, W), BF16),
        scratch_shapes=[
            pltpu.VMEM((3, 3, C, C), BF16),
            pltpu.VMEM((H, C, LANES), BF16),
            pltpu.VMEM((H, C, W_HI), BF16),
            pltpu.VMEM((H, C, W), BF16),
            pltpu.VMEM((len(MATMULS), C // 2, LANES), I32),
            pltpu.VMEM((4, C, LANES), F32),
            [pltpu.VMEM((9, C, LANES), F32)] * T_SLOTS,
            [pltpu.VMEM((4, C // 2, LANES), I32)] * E_SLOTS,
            pltpu.SMEM((1,), I32),
            pltpu.SemaphoreType.DMA((2 * CHUNKS + 1,)),
            pltpu.SemaphoreType.DMA(()),
        ],
        compiler_params=pltpu.CompilerParams(
            vmem_limit_bytes=48 * 1024 * 1024,
            disable_bounds_checks=True,
            disable_semaphore_checks=True,
        ),
    )(jnp.transpose(x.astype(BF16).reshape(H, W, C), (0, 2, 1)), w.astype(BF16))
    return jnp.transpose(y, (0, 2, 1)).reshape(1, H, W, C)
```
